```python
import os as _os
_os.environ.setdefault("JAX_PLATFORMS", "cpu")
import jax
import jax.numpy as jnp

def _softmax(x, axis=-1):
    return jax.nn.softmax(x, axis=axis)
def _gelu(x):
    return jax.nn.gelu(x, approximate=True)
def _silu(x):
    return jax.nn.silu(x)
def _sigmoid(x):
    return jax.nn.sigmoid(x)
def _layernorm(x, axis=-1, eps=1e-5):
    m = jnp.mean(x, axis=axis, keepdims=True)
    v = jnp.var(x, axis=axis, keepdims=True)
    return (x - m) / jnp.sqrt(v + eps)
def _scatter_add(tgt, idx, src, axis=0):
    return tgt.at[idx].add(src)
def _segment_sum(src, seg, n):
    return jax.ops.segment_sum(src, seg, n)
class _Rng:
    def __init__(self, key):
        self._k = key
    def _next(self):
        self._k, sub = jax.random.split(self._k)
        return sub
    def normal(self, shape):
        return jax.random.normal(self._next(), shape, dtype=jnp.bfloat16)
    def randint(self, lo, hi, shape):
        return jax.random.randint(self._next(), shape, lo, hi, dtype=jnp.int32)
    def uniform(self, shape, lo=0.0, hi=1.0):
        return jax.random.uniform(self._next(), shape, jnp.bfloat16, lo, hi)
    def permutation(self, n):
        return jax.random.permutation(self._next(), n)


kernel_name = 'standalone__layernorm_linear__sampling'

def setup_inputs():
    _rng = _Rng(jax.random.key(int.from_bytes(__import__("os").urandom(4), "little")))
    _w = (lambda a: (lambda t: t.astype(jnp.bfloat16) if jnp.issubdtype(t.dtype, jnp.floating) else t)(jnp.asarray(a)))
    B, S, D = 1024, 32, 576
    return {
        "x": _w((lambda *s: _rng.normal(s) * 0.05)(B, S, D)),
        "g": _w((lambda *s: _rng.normal(s) * 0.05)(D) + 1.0),
        "b": _w((lambda *s: _rng.normal(s) * 0.05)(D)),
        "w": _w((lambda *s: _rng.normal(s) * 0.05)(D, D)),
    }

def reference(x, g, b, w):
    return (_layernorm(x, axis=-1) * g + b) @ w
```

```python
import functools
import jax, jax.numpy as jnp
from jax import lax
import jax.experimental.pallas as pl
import jax.experimental.pallas.tpu as pltpu

EPS = 1e-5
F32, BF16, U32 = jnp.float32, jnp.bfloat16, jnp.uint32
D, H, Q = 576, 288, 144
SLOTS = Q // 16
TOFF = {i: 256 * (i - 1) for i in range(1, 8)}
E1, E2 = 1792, 1856
TOT = 1920
TE = {3: E2, 4: E1, 6: E2, 7: E1}
def _half(h): return [[(1, h + 'a'), (1, h + 'b'), (6, h + 'a'), (6, h + 'b')], [(2, h + 'a'), (2, h + 'b'), (3, h + 'a'), (3, h + 'b')], [(4, h + 'a'), (4, h + 'b'), (7, h + 'a'), (7, h + 'b')]]
ROUNDS = [[(3, 'x'), (4, 'x'), (6, 'x'), (7, 'x')]] + _half('u') + _half('l') + [[(5, 'ua'), (5, 'ub'), (5, 'la'), (5, 'lb')]]
PASSES = [p for r in ROUNDS for p in r]
SOFF = {p: Q * n for n, p in enumerate(PASSES)}
SROWS = Q * len(PASSES)

def t_rows(p):
    i, k = p
    if k == 'x': return TE[i], TOFF[i] + 192
    if k[1] == 'a': return TOFF[i], TOFF[i] + 64
    if k == 'ub' and i in TE: return TOFF[i] + 128, TE[i]
    return TOFF[i] + 128, TOFF[i] + 192

def prep_w(w_ref, g_ref, b_ref, st_ref, bias_ref):
    g = g_ref[...].astype(F32).reshape(1, D)
    b = b_ref[...].astype(F32).reshape(1, D)
    A, acc = [], None
    for t in range(5):
        if t < 4:
            w, gt, bt = w_ref[pl.ds(128 * t, 128), :], g[:, 128 * t:128 * (t + 1)], b[:, 128 * t:128 * (t + 1)]
        else:
            w = w_ref[pl.ds(512, 64), :]; w = jnp.concatenate([w, w], axis=0)
            gt = jnp.concatenate([g[:, 512:]] * 2, axis=1); bt = jnp.concatenate([b[:, 512:], jnp.zeros((1, 64), F32)], axis=1)
        wt = w.astype(F32).T
        acc = wt * bt if acc is None else acc + wt * bt
        A.append(wt * gt)
    bias_ref[...] = jnp.broadcast_to(jnp.sum(acc, axis=1, keepdims=True), bias_ref.shape)
    a1 = [v[:H] for v in A]; a2 = [v[H:] for v in A]
    S = {1: [a1[t] + a2[2 + t] for t in (0, 1)], 2: [a2[t] + a2[2 + t] for t in (0, 1)], 3: [a1[0], a1[1]], 4: [a2[2], a2[3]],
         5: [a1[t] + a1[2 + t] for t in (0, 1)], 6: [a2[t] - a1[t] for t in (0, 1)], 7: [a1[2 + t] - a2[2 + t] for t in (0, 1)]}
    SE = {3: a1[4], 4: a2[4], 6: a2[4] - a1[4], 7: a1[4] - a2[4]}
    left = lax.broadcasted_iota(jnp.int32, (Q, 128), 1) < 64
    def put(p, v): st_ref[pl.ds(SOFF[p], Q), :] = v.astype(BF16)
    for i, (sa, sb) in S.items():
        put((i, 'ua'), sa[:Q]); put((i, 'la'), sa[Q:])
        su, sl = sb[:Q], sb[Q:]
        if i in SE:
            eu, el = SE[i][:Q], SE[i][Q:]
            put((i, 'x'), jnp.where(left, el, su)); put((i, 'ub'), jnp.where(left, su, eu - el)); put((i, 'lb'), jnp.where(left, sl, sl - su))
        else:
            put((i, 'ub'), su); put((i, 'lb'), sl)

def total(parts):
    t = parts[0]()
    for p in parts[1:]: t = t + p()
    return jnp.sum(t * (1.0 / D), axis=0, keepdims=True)

def prep_steps(xload, tput, pace, rb1, rb2):
    acc = []
    for r in range(0, D, rb1):
        v = xload(r, rb1)
        p = v[0:8]
        for q in range(8, rb1, 8): p = p + v[q:q + 8]
        acc.append(pace(p, len(acc), r + rb1 == D))
        yield rb1 // 2
    mean = total(acc)
    acc = []
    for r in range(0, D, rb2):
        xc = xload(r, rb2) - mean
        v = xc * xc
        p = v[0:8]
        for q in range(8, rb2, 8): p = p + v[q:q + 8]
        acc.append(pace(p, len(acc), r + rb2 == D))
        yield rb2
    rstd = lax.rsqrt(total(acc) + EPS)
    yield 40
    m1, m2, r1, r2 = mean[:, :128], mean[:, 128:], rstd[:, :128], rstd[:, 128:]
    def y(r):
        v = xload(r, 16)
        return v[:, :128], v[:, 128:]
    for r in range(0, 64, 16):
        x31, x32 = y(512 + r)
        tput(E1 + r, (x31 - m1) * r1); tput(E2 + r, (x32 - m2) * r2)
        yield 14
    for r in list(range(192, 256, 16)) + list(range(0, 192, 16)):
        x11, x12 = y(r); x21, x22 = y(256 + r)
        t2, t5 = (x11 - m1) * r1, (x22 - m2) * r2
        t1 = t2 - t5
        tput(TOFF[2] + r, t2); tput(TOFF[5] + r, t5); tput(TOFF[1] + r, t1)
        yield 17
        t3, t4 = (x12 - x22) * r2, (x21 - x11) * r1
        tput(TOFF[3] + r, t3); tput(TOFF[4] + r, t4); tput(TOFF[6] + r, t3 - t1); tput(TOFF[7] + r, t4 + t1)
        yield 20
PREP_COST = D // 2 + D + 40 + 4 * 14 + 16 * 37

def combine(bias_ref, oput):
    x3 = yield; x4 = yield; x6 = yield; x7 = yield
    keep = []
    for h in (0, Q):
        p1 = yield; p1 = (yield) + p1
        c22 = (yield) + (x6 - p1); c22 = (yield) + c22
        p2 = (yield) + bias_ref[pl.ds(H + h, Q)]; p2 = (yield) + p2
        p3 = (yield) + x3; p3 = (yield) + p3
        oput(H + h, 1, c22 + p2 + p3)
        p4 = (yield) + x4; p4 = (yield) + p4
        oput(H + h, 0, p2 + p4)
        c11 = (yield) + (p1 + x7 + p4); c11 = (yield) + c11
        keep.append((p3, c11))
    for h, (p3, c11) in zip((0, Q), keep):
        p5 = (yield) + bias_ref[pl.ds(h, Q)]; p5 = (yield) + p5
        oput(h, 1, p3 + p5); oput(h, 0, c11 + p5)
    yield

def make(NC=8, RC=1, ramp=8, rb1=64, rb2=32, tslots=(0, 0, 1, 2, 3, 4, 5, 6), vmem=110, flags=None, q0=60, wr_per=4, nobc=True,
         nord=False, nowr=False, iters=None, nchunked=2, tab=None):
    tab = tab or (1, 1, 2, 2, 2, 1, 0, 1, 1, 0, 1)
    assert len(tab) == 3 + ramp // RC
    cum = [sum(tab[:i]) for i in range(len(tab) + 1)]
    assert cum[-1] >= 4 * nchunked
    rd_ahead = cum[-1] - 3 * nchunked
    unit = lambda q: q if q < 4 * nchunked else q // 4 + 3 * nchunked
    for j in range(ramp // RC): assert unit((j + 1) * RC) < cum[4 + j]
    NACC = D // min(rb1, rb2)
    def kern(x_hbm, g_hbm, b_hbm, w_hbm, o_hbm, xbuf, obuf, st_ref, bias_ref, isem, osem, psem):
        S, _, B = x_hbm.shape
        NQ = S * 4
        st32 = st_ref.bitcast(U32)
        rd = lambda i: pltpu.make_async_copy(x_hbm.at[i], xbuf.at[i], isem.at[4 * i])
        def rdc(q):
            sl = (q >> 2, slice(None), pl.ds(pl.multiple_of((q & 3) * 256, 256), 256))
            return pltpu.make_async_copy(x_hbm.at[sl], xbuf.at[sl], isem.at[q])
        def wr(t):
            s, c = t >> 3, t & 7
            return pltpu.make_async_copy(obuf.at[s, c], o_hbm.at[s, :, pl.ds(pl.multiple_of(c * 128, 128), 128)], osem)
        def prep(s, c, t_ref, a_ref):
            def tput(r, v): t_ref[pl.ds(r, v.shape[0]), :] = v.astype(BF16)
            def pace(p, k, last):
                if last or a_ref is None: return lambda: p
                a0 = (SROWS + 2 * TOT) // 2
                for h in range(2):
                    a_ref[pl.ds(16 * k + 8 * h, 8), :] = pltpu.bitcast(p[:, 128 * h:128 * (h + 1)], U32)
                return lambda: jnp.concatenate([pltpu.bitcast(st32[pl.ds(a0 + 16 * k + 8 * h, 8), :], F32) for h in range(2)], axis=1)
            lane = c * 256 if isinstance(c, int) else pl.multiple_of(c * 256, 256)
            return prep_steps(lambda r, n: xbuf[s, pl.ds(r, n), pl.ds(lane, 256)].astype(F32), tput, pace, rb1, rb2)
        def stage(k):
            for u in range(cum[k], cum[k + 1]):
                if u == 0 or not nord: (rdc(u) if u < 4 * nchunked else rd(u - 3 * nchunked)).start()
        def prologue(w_ref, g_ref, b_ref):
            par = [pltpu.make_async_copy(a, b, psem.at[i]) for i, (a, b) in enumerate(((g_hbm, g_ref), (b_hbm, b_ref), (w_hbm, w_ref)))]
            stage(0)
            for c in par: c.start()
            rdc(0).wait()
            stage(1)
            for _ in prep(0, 0, st_ref.at[pl.ds(SROWS, TOT)], None): pass
            for c in par: c.wait()
            stage(2)
            prep_w(w_ref, g_ref, b_ref, st_ref, bias_ref)
        pl.run_scoped(prologue, pltpu.VMEM((D, D), BF16), pltpu.VMEM((D,), BF16), pltpu.VMEM((D,), BF16))

        issued = lambda q: jnp.maximum(jnp.minimum(wr_per * (q - q0), 2 * q), 0)
        def put_writes(q):
            if nowr: return
            lo, hi = issued(q - 1), issued(q)
            for u in range(wr_per):
                @pl.when(lo + u < hi)
                def _(): wr(lo + u).start()

        def body(qs, nc, writes):
            if not nord:
                if writes:
                    for k in range(0, nc, 2):
                        ri = rd_ahead + ((qs - ramp + k) >> 1)
                        @pl.when(ri < S)
                        def _(): rd(ri).start()
                else:
                    for j in range(ramp // RC):
                        if tab[3 + j]: pl.when(qs == j * RC)(functools.partial(stage, 3 + j))
                for k in range(1, nc + 1):
                    q = qs + k
                    if not writes:
                        @pl.when(q < 4 * nchunked)
                        def _(): rdc(q).wait()
                    if nc % 4 or k % 4 == 0:
                        @pl.when((q >= 4 * nchunked) & (q < NQ) & ((q & 3) == 0))
                        def _(): rd(q >> 2).wait()
            zero = jnp.minimum(0, qs)
            if nc % 2:
                par = qs & 1
                t_st = [st_ref.at[pl.ds(pl.multiple_of(SROWS + par * TOT, 16), TOT)], st_ref.at[pl.ds(pl.multiple_of(SROWS + (1 - par) * TOT, 16), TOT)]]
                t_ld = [st32.at[pl.ds(pl.multiple_of((SROWS // 2) + par * (TOT // 2), 8), TOT // 2)], st32.at[pl.ds(pl.multiple_of((SROWS // 2) + (1 - par) * (TOT // 2), 8), TOT // 2)]]
            else:
                t_st = [st_ref.at[pl.ds(pl.multiple_of(SROWS + p * TOT + zero, 16), TOT)] for p in range(2)]
                t_ld = [st32.at[pl.ds((SROWS + p * TOT) // 2, TOT // 2)] for p in range(2)]
            a_dyn = st32.at[pl.ds(pl.multiple_of((SROWS + 2 * TOT) // 2 + zero, 8), NACC * 16)]
            def where(k, clamp=False):
                if nc % 4 == 0:
                    s = (qs >> 2) + k // 4
                    return (jnp.minimum(s, S - 1) if clamp else s), k % 4
                q = jnp.minimum(qs + k, NQ - 1)
                return q >> 2, q & 3
            NR = nc * len(ROUNDS)
            dl = [(len(ROUNDS) * (c + 1) - 1) * SLOTS + tslots[0] for c in range(nc - 1)] + [NR * SLOTS]
            def tload(G, v):
                rows = [t_rows(p)[v // 4] + 16 * (v % 4) for p in ROUNDS[G % len(ROUNDS)]]
                got = {}
                for r in rows:
                    if r not in got: got[r] = t_ld[(G // len(ROUNDS)) % 2][pl.ds(r // 2, 8), :]
                return [got[r] for r in rows]
            cur, pg, spent = -1, None, 0
            tnext = [tload(0, v) for v in range(8)]
            for G in range(NR):
                rnd = ROUNDS[G % len(ROUNDS)]
                tcur, tnext = tnext, []
                lhs = []
                for i in range(SLOTS):
                    lhs.append([st32[pl.ds((SOFF[p] + 16 * i) // 2, 8), :] for p in rnd])
                    slot = G * SLOTS + i
                    if cur < 0 or (slot >= dl[cur] and cur + 1 < nc):
                        if pg is not None:
                            for _ in pg: pass
                        cur += 1
                        pg, spent = prep(*where(cur + 1, cur + 1 == nc), t_st[(cur + 1) % 2], a_dyn), 0
                    if G + 1 < NR:
                        for v in range(8):
                            if tslots[v] == i: tnext.insert(0, tload(G + 1, 7 - v))
                    lo = dl[cur - 1] if cur else 0
                    goal = PREP_COST * (slot + 1 - lo) / (dl[cur] - lo)
                    while spent < goal:
                        cst = next(pg, None)
                        if cst is None: break
                        spent += cst
                if G % len(ROUNDS) == 0:
                    k = G // len(ROUNDS)
                    if writes: put_writes(qs + k)
                    s, c = where(k)
                    def oput(r, jj, v, s=s, c=c): obuf[s, 2 * c + jj, pl.ds(r, Q), :] = v.astype(BF16)
                    comb = combine(bias_ref, oput); next(comb)
                for m in range(4):
                    a = pltpu.bitcast(jnp.concatenate([v[m] for v in lhs], axis=0), BF16)
                    t = pltpu.bitcast(jnp.concatenate([v[m] for v in tcur], axis=0), BF16)
                    comb.send(jnp.dot(a, t, preferred_element_type=F32))
            for _ in pg: pass
        assert ramp % RC == 0 and (NQ - ramp) % NC == 0 and q0 >= ramp and 4 * nchunked <= ramp + 1
        if ramp: lax.fori_loop(0, ramp // RC, lambda j, _: body(j * RC, RC, False), None)
        lax.fori_loop(0, iters or (NQ - ramp) // NC, lambda j, _: body(ramp + j * NC, NC, True), None)
        put_writes(NQ)
        if nowr: wr(0).start(); wr(0).wait()
        else: pltpu.make_async_copy(obuf, obuf, osem).wait()

    def fn(x, g, b, w):
        B, S, _ = x.shape
        xt = jnp.transpose(x, (1, 2, 0))
        out = pl.pallas_call(
            kern,
            in_specs=[pl.BlockSpec(memory_space=pl.ANY)] * 4,
            out_specs=pl.BlockSpec(memory_space=pl.ANY),
            out_shape=jax.ShapeDtypeStruct((S, D, B), x.dtype),
            scratch_shapes=[pltpu.VMEM((S, D, B), BF16), pltpu.VMEM((S, B // 128, D, 128), BF16), pltpu.VMEM((SROWS + 2 * TOT + NACC * 32, 128), BF16), pltpu.VMEM((D, 128), F32),
                            pltpu.SemaphoreType.DMA((4 * S,)), pltpu.SemaphoreType.DMA, pltpu.SemaphoreType.DMA((3,))],
            compiler_params=pltpu.CompilerParams(vmem_limit_bytes=vmem * 1024 * 1024, flags=flags, disable_bounds_checks=nobc),
        )(xt, g, b, w)
        return jnp.transpose(out, (2, 0, 1))
    return fn


@jax.jit
def pallas_standalone__layernorm_linear__sampling_kernel(x, g, b, w):
    return make(NC=8, q0=56)(x, g, b, w)
```

```python
import functools

import jax
import jax.numpy as jnp
from jax import lax
import jax.experimental.pallas as pl
import jax.experimental.pallas.tpu as pltpu

_EPS = 1e-5
_F32, _BF16, _U32 = jnp.float32, jnp.bfloat16, jnp.uint32

_B, _S, _D = 1024, 32, 576
_CHUNK = 256
_CHUNKS = _B * _S // _CHUNK
_SLOTS = _D // 4 // 16
_STAGES = ((2, 2), (4, 4), (12, 9))
_MEAN_ROWS, _VAR_ROWS = 64, 32

_ONE_LEVEL = (1, 3, 4, 6, 7)
_TWO_LEVEL = (2, 5)


def _chunk_passes(c):
    passes = [(i, "x", c) for i in (3, 4, 6, 7)]
    for half in "ul":
        passes += [(i, half + t, c) for i in (1, 6, 3, 4) for t in "ab"]
    return passes + [(7, kind, c) for kind in ("ua", "ub", "la", "lb")]


_INNER = [(2, m, 0) for m in (1, 2, 3, 6, 4, 5, 7)] + [(5, m, 0) for m in (1, 2, 3, 4, 5)]
_EDGE = [(5, 7, 0), (5, 6, 0)]
_ORDER = (
    _INNER + _chunk_passes(0) + _chunk_passes(1) + _EDGE,
    _EDGE + _INNER + _chunk_passes(0) + _chunk_passes(1),
)
_PASSES = len(_ORDER[0])

_W_CELL = {key: _SLOTS * n for n, key in enumerate(dict.fromkeys(p[:2] for p in _ORDER[0]))}
_W_CELLS = -(-_SLOTS * len(_W_CELL) // 4) * 4
_T_CELL = {i: 16 * n for n, i in enumerate(_ONE_LEVEL)}
_TAIL_CELL = (16 * len(_ONE_LEVEL), 16 * len(_ONE_LEVEL) + 4)
_TAIL_OF = {3: _TAIL_CELL[1], 4: _TAIL_CELL[0], 6: _TAIL_CELL[1], 7: _TAIL_CELL[0]}
_CHUNK_CELLS = 16 * len(_ONE_LEVEL) + 8
_U_CELL = {
    (i, m): 2 * _CHUNK_CELLS + 8 * (7 * n + m - 1)
    for n, i in enumerate(_TWO_LEVEL)
    for m in range(1, 8)
}
_PAIR_CELLS = 2 * _CHUNK_CELLS + 8 * len(_U_CELL)
_SUM_BASE = _W_CELLS + 2 * _PAIR_CELLS
_SUMS = _D // min(_MEAN_ROWS, _VAR_ROWS) + 2

_LOAD_SLOT = (0, 0, 1, 2, 3, 4, 5, 6)
_RSQRT_WAIT = 100
_PREP_COST = 2 * (_D // 2 + _D + 4 * 14) + _RSQRT_WAIT + 32 * 35 + 16 * 41

_WIDE_COPIES, _WIDE_PER_PAIR, _WIDE_DELAY = 224, 9, 279
_LAST_TILES = {-12: (-32, -24), -8: (-24, -16), -6: (-16, -12), -5: (-12, -10),
               -4: (-10, -8), -2: (-8, -4), -1: (-4, -2), 0: (-2, 0)}


def _cell(n):
    return pl.ds(8 * (n // 2), 8), pl.ds(128 * (n % 2), 128)


def _put_cell(ref, n, value):
    ref[_cell(n)] = pltpu.bitcast(value.astype(_BF16), _U32)


def _activation_cells(p):
    i, kind, c = p
    if i in _TWO_LEVEL:
        return [_U_CELL[i, kind] + v for v in range(8)]
    if kind == "x":
        halves = _TAIL_OF[i], _T_CELL[i] + 12
    elif kind[1] == "a":
        halves = _T_CELL[i], _T_CELL[i] + 4
    elif kind == "ub" and i in _TAIL_OF:
        halves = _T_CELL[i] + 8, _TAIL_OF[i]
    else:
        halves = _T_CELL[i] + 8, _T_CELL[i] + 12
    return [c * _CHUNK_CELLS + h + v for h in halves for v in range(4)]


def _strassen_lhs(a11, a12, a21, a22):
    return {1: a11 + a22, 2: a21 + a22, 3: a11, 4: a22, 5: a11 + a12, 6: a21 - a11, 7: a12 - a22}


def _prepare_weights(w_ref, g_ref, b_ref, ops_ref, bias_ref):
    g = g_ref[...].astype(_F32).reshape(1, _D)
    b = jnp.broadcast_to(b_ref[...].astype(_F32).reshape(1, _D), (16, _D)).astype(_BF16)
    bias = jnp.dot(b, w_ref[...], preferred_element_type=_F32)[0:1]
    g = [g[:, 128 * t:128 * (t + 1)] for t in range(4)] + [jnp.concatenate([g[:, 512:]] * 2, axis=1)]
    left = lax.broadcasted_iota(jnp.int32, (16, 128), 1) < 64

    def operands(a1, a2):
        tiles = [_strassen_lhs(a1[t], a1[2 + t], a2[t], a2[2 + t]) for t in (0, 1)]
        return tiles, {3: a1[4], 4: a2[4], 6: a2[4] - a1[4], 7: a1[4] - a2[4]}

    for n0 in range(0, _D, 128):
        cols = pl.ds(n0, min(128, _D - n0))
        w = [w_ref[pl.ds(128 * t, 128), cols] for t in range(4)]
        w.append(jnp.concatenate([w_ref[pl.ds(512, 64), cols]] * 2, axis=0))
        wt = [v.T.astype(_F32) for v in w]
        for f in range(0, cols.size, 64):
            slot = (n0 + f) // 64
            a1u, a1l, a2u, a2l = (
                [wt[t][f + 16 * role:f + 16 * (role + 1)] * g[t] for t in range(5)] for role in range(4)
            )
            (up, up_tail), (lo, lo_tail) = operands(a1u, a2u), operands(a1l, a2l)
            for i in range(1, 8):
                ua, ub, la, lb = up[0][i], up[1][i], lo[0][i], lo[1][i]
                if i in _TWO_LEVEL:
                    tiles = {m: -v if m >= 6 else v for m, v in _strassen_lhs(ua, ub, la, lb).items()}
                elif i in up_tail:
                    tiles = {
                        "ua": ua,
                        "la": la,
                        "x": jnp.where(left, lo_tail[i], ub),
                        "ub": jnp.where(left, ub, up_tail[i] - lo_tail[i]),
                        "lb": jnp.where(left, lb, lb - ub),
                    }
                else:
                    tiles = {"ua": ua, "la": la, "ub": ub, "lb": lb}
                for kind, value in tiles.items():
                    _put_cell(ops_ref, _W_CELL[i, kind] + slot, value)
    bias_ref[...] = jnp.broadcast_to(bias, (128, _D)).T


def _tree_sum(vs):
    while len(vs) > 1:
        vs = [vs[i] + vs[i + 1] if i + 1 < len(vs) else vs[i] for i in range(0, len(vs), 2)]
    return vs[0]


def _prepare_activations(load, put, park):
    def partial_average(term, rows, cost, c):
        parts = []
        for r in range(0, _D, rows):
            v = term(r)
            part = _tree_sum([v[k:k + 8] for k in range(0, rows, 8)])
            parts.append(park(len(parts), part) if r + rows < _D else lambda: part)
            yield cost
        return park(_SUMS - 2 + c, _tree_sum([p() for p in parts]) * (1.0 / _D))

    def finish(parked):
        v = parked()
        return jnp.broadcast_to(jnp.sum(v, axis=0, keepdims=True), v.shape)

    def deviation(c, r):
        return jnp.square(load(c, r, _VAR_ROWS) - jnp.tile(mean[c], (_VAR_ROWS // 8, 1)))

    s0 = yield from partial_average(lambda r: load(0, r, _MEAN_ROWS), _MEAN_ROWS, _MEAN_ROWS // 2, 0)
    s1 = yield from partial_average(lambda r: load(1, r, _MEAN_ROWS), _MEAN_ROWS, _MEAN_ROWS // 2, 1)
    mean = [finish(s0)]
    s0 = yield from partial_average(lambda r: deviation(0, r), _VAR_ROWS, _VAR_ROWS, 0)
    mean.append(finish(s1))
    s1 = yield from partial_average(lambda r: deviation(1, r), _VAR_ROWS, _VAR_ROWS, 1)
    mean = [jnp.tile(v, (2, 1)) for v in mean]
    rstd = []
    for c, var in enumerate((s0, s1)):
        rstd.append(jnp.tile(lax.rsqrt(finish(var) + _EPS), (2, 1)))
        yield c * _RSQRT_WAIT
        for n in range(4):
            v = (load(c, 512 + 16 * n, 16) - mean[c]) * rstd[c]
            put(c * _CHUNK_CELLS + _TAIL_CELL[0] + n, v[:, :128])
            put(c * _CHUNK_CELLS + _TAIL_CELL[1] + n, v[:, 128:])
            yield 14

    def tile(v, h):
        return v[:, 128 * h:128 * (h + 1)]

    for c in range(2):
        m1, m2, r1, r2 = tile(mean[c], 0), tile(mean[c], 1), tile(rstd[c], 0), tile(rstd[c], 1)
        for n in range(16):
            v1, v2 = load(c, 16 * n, 16), load(c, 256 + 16 * n, 16)
            x11, x12, x21, x22 = tile(v1, 0), tile(v1, 1), tile(v2, 0), tile(v2, 1)
            t1 = (x11 - m1) * r1 - (x22 - m2) * r2
            t3, t4 = (x12 - x22) * r2, (x21 - x11) * r1
            for i, v in ((1, t1), (3, t3), (4, t4)):
                put(c * _CHUNK_CELLS + _T_CELL[i] + n, v)
            yield 22
            for i, v in ((6, t3 - t1), (7, t4 + t1)):
                put(c * _CHUNK_CELLS + _T_CELL[i] + n, v)
            yield 13
    for h, i in enumerate(_TWO_LEVEL):
        for n in range(8):
            (b11, b12), (b21, b22) = (
                [
                    (tile(load(c, 256 * h + 128 * t + 16 * n, 16), h) - tile(mean[c], h)) * tile(rstd[c], h)
                    for c in range(2)
                ]
                for t in range(2)
            )
            for m, v in ((2, b11), (5, b22), (1, b11 - b22)):
                put(_U_CELL[i, m] + n, v)
            yield 20
            for m, v in ((3, b12 - b22), (4, b21 - b11), (6, b12 - b11), (7, b21 - b22)):
                put(_U_CELL[i, m] + n, v)
            yield 21


def _combine(order, bias_ref, put):
    m, shared, late, c11, c12 = {}, {}, {}, {}, {}
    negated = {(0, 0): 7, (1, 1): 6}

    def bias(role):
        return jnp.concatenate([bias_ref[pl.ds(64 * s + 16 * role, 16), :] for s in range(_SLOTS)], axis=0)

    def second_level(i, h, c):
        if (h, c) == (0, 0):
            v = m[i, 1] + m[i, 4] + m[i, 5]
        elif (h, c) == (1, 1):
            v = m[i, 2] + m[i, 3] - m[i, 1]
        else:
            v = m[i, 3] + m[i, 5] if c else m[i, 2] + m[i, 4]
        last = (i, negated.get((h, c)))
        return v - m[last] if last in m else v

    for i, kind, c in order:
        if i in _TWO_LEVEL:
            v = yield
            if kind in (2, 5):
                v = v + bias(2 * (i == 2) + (kind == 2))
            m[i, kind] = v
            if (i, kind) in late:
                chunk, h, left, right = late.pop((i, kind))
                put(chunk, h, left - v, right - v)
        elif kind == "x":
            shared[i] = yield
        elif kind[1] == "a":
            h = "ul".index(kind[0])
            if i == 1:
                acc = yield
                continue
            start = shared[6] - p1 if i == 6 else shared[7] + c11[h] if i == 7 else shared[i]
            acc = (yield) + start
        else:
            p = (yield) + acc
            if i == 1:
                p1 = p
            elif i == 6:
                c22 = p
            elif i == 3:
                p3 = p
            elif i == 4:
                p2 = second_level(2, h, c)
                put(c, 2 + h, p2 + p, p2 + c22 + p3)
                p5 = second_level(5, h, c)
                c11[h], c12[h] = p5 + p1 + p, p5 + p3
            elif (h, c) in negated and (5, negated[h, c]) not in m:
                late[5, negated[h, c]] = (c, h, p, c12[h])
            else:
                put(c, h, p, c12[h])
    yield


def _kernel(x_hbm, g_hbm, b_hbm, w_hbm, o_hbm, x_ref, o_ref, ops_ref, bias_ref, x_sem, o_sem, p_sem):
    def read_slice(s):
        return pltpu.make_async_copy(x_hbm.at[s], x_ref.at[s], x_sem.at[s + 1])

    def read_first(half):
        part = (0, slice(None), pl.ds(half * _B // 2, _B // 2))
        return pltpu.make_async_copy(x_hbm.at[part], x_ref.at[part], x_sem.at[half])

    def requested(q):
        return (q >> 1) + 2

    def write_strided(period, first, count, offset):
        def view(ref):
            groups = ref.reshape(_S * _D // (16 * period), period, 16, _B)
            return groups.at[pl.ds(first, count), pl.ds(offset, 1)]

        return pltpu.make_async_copy(view(o_ref), view(o_hbm), o_sem)

    def write_wide(q):
        for u in range(_WIDE_PER_PAIR):
            n = _WIDE_PER_PAIR * (q >> 1) - _WIDE_DELAY + u

            @pl.when((n >= 0) & (n < _WIDE_COPIES))
            def _():
                write_strided(32, (n >> 5) * 4, 4, ((n & 1) << 4) | ((n & 31) >> 1)).start()

    def write_last(done):
        if done == _CHUNKS - 16:
            for offset in range(16):
                write_strided(16, 56, 7, offset).start()
        for t in range(*_LAST_TILES.get(done - _CHUNKS, (0, 0))):
            s, col = divmod(2 * _CHUNKS + t, _B // 128)
            part = (s, slice(None), pl.ds(col * 128, 128))
            pltpu.make_async_copy(o_ref.at[part], o_hbm.at[part], o_sem).start(priority=t % 2)

    def cells(row, count):
        row = row if isinstance(row, int) else pl.multiple_of(row, 16)
        return ops_ref.at[pl.ds(row, 4 * count)]

    def lanes(first):
        starts = [(first + c) * _CHUNK for c in range(2)]
        return [pl.ds(v if isinstance(v, int) else pl.multiple_of(v, _CHUNK), _CHUNK) for v in starts]

    def prepare(s, first, tiles_ref, sums_ref):
        cols = lanes(first)

        def park(n, value):
            sums_ref[pl.ds(8 * n, 8), :] = pltpu.bitcast(value, _U32)
            return lambda: pltpu.bitcast(ops_ref[pl.ds(4 * _SUM_BASE + 8 * n, 8), :], _F32)

        return _prepare_activations(
            lambda c, r, rows: x_ref[s, pl.ds(r, rows), cols[c]].astype(_F32),
            functools.partial(_put_cell, tiles_ref),
            park,
        )

    def prologue(w_ref, g_ref, b_ref):
        params = [
            pltpu.make_async_copy(src, dst, p_sem.at[n])
            for n, (src, dst) in enumerate(((g_hbm, g_ref), (b_hbm, b_ref), (w_hbm, w_ref)))
        ]
        for copy in params:
            copy.start()
        read_first(0).start()
        for copy in params:
            copy.wait()
        read_first(1).start()
        _prepare_weights(w_ref, g_ref, b_ref, ops_ref, bias_ref)
        read_first(0).wait()
        pieces = prepare(0, 0, cells(4 * _W_CELLS, _PAIR_CELLS), cells(4 * _SUM_BASE, 2 * _SUMS))
        for n, _ in enumerate(pieces, 1):
            if n == 2 * (_D // _MEAN_ROWS + _D // _VAR_ROWS):
                read_slice(1).start()
        read_first(1).wait()

    def step(q, chunks, has_writes):
        pairs = chunks // 2
        for k in range(2, chunks + 1, 2):
            if chunks % 4 or k % 4 == 0:

                @pl.when((((q + k) & 3) == 0) & (q + k < _CHUNKS))
                def _():
                    read_slice((q + k) >> 2).wait()

        zero = jnp.minimum(0, q + 16)
        parity = (q >> 1) & 1 if pairs % 2 else 0
        rows = [4 * _W_CELLS + ((p + parity) & 1) * (4 * _PAIR_CELLS) for p in range(2)]
        tiles_out = [cells(row + zero, _PAIR_CELLS) for row in rows]
        tiles_in = [cells(row, _PAIR_CELLS) for row in rows]
        sums_out = cells(4 * _SUM_BASE + zero, 2 * _SUMS)

        def locate(k):
            if chunks % 4:
                return (q + 2 * k) >> 2, (q + 2 * k) & 2
            s = (q >> 2) + k // 2
            return jnp.minimum(s, _S - 1) if k == pairs else s, k % 2 * 2

        def write(k):
            if not has_writes:
                return
            if k % 2 == 0:
                write_wide(q + k)
            for done in range(_CHUNKS - chunks + k, _CHUNKS - 17, -chunks):
                if done == _CHUNKS - 16 or done - _CHUNKS in _LAST_TILES:
                    pl.when(q + k == done)(functools.partial(write_last, done))

        passes = [(k, p) for k in range(pairs) for p in _ORDER[k % 2]]
        rounds = [passes[n:n + 4] for n in range(0, len(passes), 4)]
        window = [0] + [(_PASSES * k // 4 - 1) * _SLOTS + _LOAD_SLOT[0] for k in range(1, pairs)]
        window.append(len(rounds) * _SLOTS)

        def load_tiles(round_, v):
            keys = [(k % 2, _activation_cells(p)[v]) for k, p in round_]
            loaded = {key: tiles_in[key[0]][_cell(key[1])] for key in dict.fromkeys(keys)}
            return [loaded[key] for key in keys]

        upcoming = [load_tiles(rounds[0], v) for v in range(8)]
        write(0)
        current, pieces, spent = -1, iter(()), 0
        for r, round_ in enumerate(rounds):
            tiles, upcoming, weights = upcoming, [], []
            for slot in range(_SLOTS):
                weights.append([ops_ref[_cell(_W_CELL[p[:2]] + slot)] for _, p in round_])
                now = r * _SLOTS + slot
                if now == window[current + 1]:
                    for _ in pieces:
                        pass
                    current, spent = current + 1, 0
                    pieces = prepare(*locate(current + 1), tiles_out[(current + 1) % 2], sums_out)
                if r + 1 < len(rounds):
                    for v in range(8):
                        if _LOAD_SLOT[v] == slot:
                            upcoming.insert(0, load_tiles(rounds[r + 1], 7 - v))
                start, end = window[current:current + 2]
                while spent < _PREP_COST * (now + 1 - start) / (end - start):
                    spent += next(pieces, _PREP_COST)
            for mxu, (k, p) in enumerate(round_):
                n = (4 * r + mxu) % _PASSES
                if n == 0:
                    s, first = locate(k)

                    def put(c, role, left, right, s=s, cols=lanes(first)):
                        y = jnp.concatenate([left, right], axis=1)
                        for slot in range(_SLOTS):
                            value = y[16 * slot:16 * (slot + 1)].astype(o_ref.dtype)
                            o_ref[s, pl.ds(64 * slot + 16 * role, 16), cols[c]] = value

                    combine = _combine(_ORDER[k % 2], bias_ref, put)
                    next(combine)
                lhs = pltpu.bitcast(jnp.concatenate([v[mxu] for v in weights], axis=0), _BF16)
                rhs = pltpu.bitcast(jnp.concatenate([v[mxu] for v in tiles], axis=0), _BF16)
                combine.send(jnp.dot(lhs, rhs, preferred_element_type=_F32))
                if k % 2 and p == _chunk_passes(0)[-1]:
                    write(2 * k + 1)
                if n == _PASSES - 1 and k + 1 < pairs:
                    write(2 * k + 2)
        for _ in pieces:
            pass
        for k in range(pairs):
            s = requested(q + chunks) + k

            @pl.when(s < _S)
            def _():
                read_slice(s).start()

    pl.run_scoped(
        prologue, pltpu.VMEM((_D, _D), _BF16), pltpu.VMEM((_D,), _BF16), pltpu.VMEM((_D,), _BF16)
    )
    q = previous = 0
    for n, (chunks, steps) in enumerate(_STAGES, 1):
        for s in range(requested(q + previous), requested(q + chunks)):
            read_slice(s).start()
        body = functools.partial(step, chunks=chunks, has_writes=n == len(_STAGES))
        lax.fori_loop(0, steps, lambda j, _, q=q, chunks=chunks, body=body: body(q + j * chunks), None)
        q, previous = q + chunks * steps, chunks
    write_last(_CHUNKS)
    pltpu.make_async_copy(o_ref, o_hbm, o_sem).wait()


@jax.jit
def pallas_standalone__layernorm_linear__sampling_kernel(
    x: jax.Array,
    g: jax.Array,
    b: jax.Array,
    w: jax.Array,
):
    assert x.shape == (_B, _S, _D) and w.shape == (_D, _D) and x.dtype == w.dtype == _BF16
    out = pl.pallas_call(
        _kernel,
        in_specs=[pl.BlockSpec(memory_space=pl.ANY)] * 4,
        out_specs=pl.BlockSpec(memory_space=pl.ANY),
        out_shape=jax.ShapeDtypeStruct((_S, _D, _B), x.dtype),
        scratch_shapes=[
            pltpu.VMEM((_S, _D, _B), _BF16),
            pltpu.VMEM((_S, _D, _B), _BF16),
            pltpu.VMEM((4 * _SUM_BASE + 8 * _SUMS, 256), _U32),
            pltpu.VMEM((_D, 128), _F32),
            pltpu.SemaphoreType.DMA((_S + 1,)),
            pltpu.SemaphoreType.DMA,
            pltpu.SemaphoreType.DMA((3,)),
        ],
        compiler_params=pltpu.CompilerParams(
            vmem_limit_bytes=100 * 1024 * 1024,
            disable_bounds_checks=True,
            disable_semaphore_checks=True,
        ),
    )(jnp.transpose(x, (1, 2, 0)), g, b, w)
    return jnp.transpose(out, (2, 0, 1))
```
